```python
import jax
import jax.numpy as jnp

def _softmax(x, axis=-1):
    return jax.nn.softmax(x, axis=axis)
def _gelu(x):
    return jax.nn.gelu(x, approximate=True)
def _silu(x):
    return jax.nn.silu(x)
def _sigmoid(x):
    return jax.nn.sigmoid(x)
def _layernorm(x, axis=-1, eps=1e-5):
    m = jnp.mean(x, axis=axis, keepdims=True)
    v = jnp.var(x, axis=axis, keepdims=True)
    return (x - m) / jnp.sqrt(v + eps)
def _scatter_add(tgt, idx, src, axis=0):
    return tgt.at[idx].add(src)
def _segment_sum(src, seg, n):
    return jax.ops.segment_sum(src, seg, n)
class _Rng:
    def __init__(self, key):
        self._k = key
    def _next(self):
        self._k, sub = jax.random.split(self._k)
        return sub
    def normal(self, shape):
        return jax.random.normal(self._next(), shape, dtype=jnp.bfloat16)
    def randint(self, lo, hi, shape):
        return jax.random.randint(self._next(), shape, lo, hi, dtype=jnp.int32)
    def uniform(self, shape, lo=0.0, hi=1.0):
        return jax.random.uniform(self._next(), shape, jnp.bfloat16, lo, hi)
    def permutation(self, n):
        return jax.random.permutation(self._next(), n)


kernel_name = 'parallel_sum__gqa_block_cached__moe_arch_mod__decode'

def setup_inputs():
    _rng = _Rng(jax.random.key(int.from_bytes(__import__("os").urandom(4), "little")))
    _w = (lambda a: (lambda t: t.astype(jnp.bfloat16) if jnp.issubdtype(t.dtype, jnp.floating) else t)(jnp.asarray(a)))
    def _A_setup():
        B, Sq, D = 1, 1, 448
        Hq, Hkv, Sk, Dh = 16, 8, 65536, 256
        assert Hq % Hkv == 0, (Hq, Hkv)
        return {
            "x": _w((lambda *s: _rng.normal(s) * 0.05)(B, Sq, D)),
            "k_cache": _w((lambda *s: _rng.normal(s) * 0.05)(B, Hkv, Sk, Dh)),
            "v_cache": _w((lambda *s: _rng.normal(s) * 0.05)(B, Hkv, Sk, Dh)),
            "wq": _w((lambda *s: _rng.normal(s) * 0.05)(D, Hq * Dh) * (D ** -0.5)),
            "wo": _w((lambda *s: _rng.normal(s) * 0.05)(Hq * Dh, D) * ((Hq * Dh) ** -0.5)),
        }
    _A_in = _A_setup()

    def _B_setup():
        B, S, D, F, C = 1, 1, 448, 1792, 1
        return {
            "x": _w((lambda *s: _rng.normal(s) * 0.05)(B, S, D)),
            "w_r": _w((lambda *s: _rng.normal(s) * 0.05)(D)),
            "w_gate": _w((lambda *s: _rng.normal(s) * 0.05)(D, F)),
            "w_up": _w((lambda *s: _rng.normal(s) * 0.05)(D, F)),
            "w_down": _w((lambda *s: _rng.normal(s) * 0.05)(F, D)),
        }
    _B_in = _B_setup()

    return {
        "A_x": _A_in["x"],
        "A_k_cache": _A_in["k_cache"],
        "A_v_cache": _A_in["v_cache"],
        "A_wq": _A_in["wq"],
        "A_wo": _A_in["wo"],
        "B_x": _B_in["x"],
        "B_w_r": _B_in["w_r"],
        "B_w_gate": _B_in["w_gate"],
        "B_w_up": _B_in["w_up"],
        "B_w_down": _B_in["w_down"],
    }

def reference(A_x, A_k_cache, A_v_cache, A_wq, A_wo, B_x, B_w_r, B_w_gate, B_w_up, B_w_down):
    def _A_ref(x, k_cache, v_cache, wq, wo):
        B, Sq, D = x.shape
        Hq, Dh = 16, 256
        Hkv = k_cache.shape[1]
        rep = Hq // Hkv
        q = (lambda x, *d: x.transpose(*d))((x @ wq).reshape(B, Sq, Hq, Dh), 0, 2, 1, 3)
        k = jnp.repeat(k_cache, rep, axis=1)
        v = jnp.repeat(v_cache, rep, axis=1)
        scores = jnp.einsum("bhqd,bhkd->bhqk", q, k) * (Dh ** -0.5)
        p = _softmax(scores, axis=-1)
        o = jnp.einsum("bhqk,bhkd->bhqd", p, v)
        return (lambda x, *d: x.transpose(*d))(o, 0, 2, 1, 3).reshape(B, Sq, Hq * Dh) @ wo

    def _B_ref(x, w_r, w_gate, w_up, w_down):
        B, S, D = x.shape
        C = 1
        r = x @ w_r
        idx = jnp.argsort(-r, axis=-1)[:, :C]
        idx_e = jnp.repeat(idx.reshape(B, C, 1), D, axis=2)
        x_sel = jnp.take_along_axis(x, idx_e, axis=1)
        g = _silu(x_sel @ w_gate)
        u = x_sel @ w_up
        y = (g * u) @ w_down
        r_sel = _sigmoid(jnp.take_along_axis(r, idx, axis=1))
        y = y * r_sel.reshape(B, C, 1)
        b_off = (jnp.arange(B) * S).reshape(B, 1)
        flat_idx = (idx + b_off).reshape(B * C)
        zero = (x * 0.0).reshape(B * S, D)
        upd = _scatter_add(zero, flat_idx, y.reshape(B * C, D), axis=0)
        return x + upd.reshape(B, S, D)

    x = A_x
    xn = _layernorm(x, axis=-1)
    return x + _A_ref(xn, A_k_cache, A_v_cache, A_wq, A_wo) + _B_ref(xn, B_w_r, B_w_gate, B_w_up, B_w_down)
```

```python
import functools
import jax
import jax.numpy as jnp
from jax import lax
import jax.experimental.pallas as pl
import jax.experimental.pallas.tpu as pltpu

D = 448
HQ = 16
HKV = 8
DH = 256
SK = 65536
F = 1792


def _make(CH=64, BS=2048, NBUF=4, do_dma=True, do_compute=True):
    G = BS // CH
    NC = SK // BS
    TOT = HKV * NC

    def kernel(x_hbm, k_hbm, v_hbm, wq_hbm, woT_hbm, wr_hbm, wg_hbm, wu_hbm, wdT_hbm, o_ref,
               x_v, wr_v, wq_v, woT_v, wg_v, wu_v, wdT_v, kb, vb, q_s, o_s, sk, sv, sw):
        def start(i, slot):
            g = i // NC
            j = i % NC
            for c in range(G):
                pltpu.make_async_copy(k_hbm.at[0, g, pl.ds(j * BS + c * CH, CH), :],
                                      kb.at[slot, pl.ds(c * CH, CH), :], sk.at[slot]).start(priority=0)
                pltpu.make_async_copy(v_hbm.at[0, g, pl.ds(j * BS + c * CH, CH), :],
                                      vb.at[slot, pl.ds(c * CH, CH), :], sv.at[slot]).start(priority=1)

        def wait(slot):
            pltpu.make_async_copy(kb.at[slot], kb.at[slot], sk.at[slot]).wait()
            pltpu.make_async_copy(vb.at[slot], vb.at[slot], sv.at[slot]).wait()

        small = [(x_hbm, x_v), (wr_hbm, wr_v)]
        for n, (a, b) in enumerate(small):
            pltpu.make_async_copy(a, b, sw.at[n]).start()
        n = 0
        for r in range(D // 16):
            for c in range(4):
                pltpu.make_async_copy(wq_hbm.at[pl.ds(r * 16, 16), pl.ds(c * 1024, 1024)],
                                      wq_v.at[pl.ds(r * 16, 16), pl.ds(c * 1024, 1024)], sw.at[2]).start(priority=n % 2)
                n += 1
        if do_dma:
            for s in range(NBUF - 1):
                start(s, s)
        for n, (a, b) in enumerate(small):
            pltpu.make_async_copy(a, b, sw.at[n]).wait()
        x = x_v[...].astype(jnp.float32)
        mu = jnp.mean(x, axis=-1, keepdims=True)
        xc = x - mu
        var = jnp.mean(xc * xc, axis=-1, keepdims=True)
        xn = (xc / jnp.sqrt(var + 1e-5)).astype(jnp.bfloat16)
        xb = jnp.broadcast_to(xn, (8, D))
        pltpu.make_async_copy(wq_v, wq_v, sw.at[2]).wait()
        q = jnp.dot(xb, wq_v[...], preferred_element_type=jnp.float32)
        q = q.astype(jnp.bfloat16).astype(jnp.float32) * (DH ** -0.5)
        row = lax.broadcasted_iota(jnp.int32, (8, DH), 0)
        for h in range(HKV):
            q_s[h] = jnp.where(row == 0, q[:, h * 512:h * 512 + 256], q[:, h * 512 + 256:h * 512 + 512]).astype(jnp.bfloat16)

        def wcopies():
            cps = []
            for (src, dst, sem, R, C, cw) in [(wg_hbm, wg_v, 3, D, F, 896), (wu_hbm, wu_v, 4, D, F, 896),
                                              (wdT_hbm, wdT_v, 5, D, F, 896), (woT_hbm, woT_v, 6, D, HQ * DH, 1024)]:
                n = 0
                for r in range(R // 16):
                    for c in range(C // cw):
                        cps.append((pltpu.make_async_copy(src.at[pl.ds(r * 16, 16), pl.ds(c * cw, cw)],
                                                          dst.at[pl.ds(r * 16, 16), pl.ds(c * cw, cw)], sw.at[sem]), n % 2))
                        n += 1
            return cps

        def body(i, carry):
            m_prev, l_prev, acc = carry
            slot = i % NBUF
            g = i // NC
            j = i % NC
            if do_dma:
                wait(slot)

                @pl.when(i + NBUF - 1 < TOT)
                def _():
                    start(i + NBUF - 1, (i + NBUF - 1) % NBUF)
            if do_compute:
                first = j == 0
                m_prev = jnp.where(first, -jnp.inf, m_prev)
                l_prev = jnp.where(first, 0.0, l_prev)
                acc = jnp.where(first, 0.0, acc)
                s = lax.dot_general(q_s[g], kb[slot], (((1,), (1,)), ((), ())), preferred_element_type=jnp.float32)
                m_new = jnp.maximum(m_prev, jnp.max(s, axis=-1, keepdims=True))
                alpha = jnp.exp(m_prev - m_new)
                p = jnp.exp(s - m_new)
                l_new = alpha * l_prev + jnp.sum(p, axis=-1, keepdims=True)
                acc = alpha * acc + jnp.dot(p.astype(jnp.bfloat16), vb[slot], preferred_element_type=jnp.float32)

                @pl.when(j == NC - 1)
                def _():
                    o = acc / l_new
                    o_s[0:1, pl.ds(pl.multiple_of(g * 512, 512), 256)] = o[0:1]
                    o_s[0:1, pl.ds(pl.multiple_of(g * 512 + 256, 256), 256)] = o[1:2]
                return m_new, l_new, acc
            return carry

        init = (jnp.zeros((8, 1), jnp.float32), jnp.zeros((8, 1), jnp.float32), jnp.zeros((8, DH), jnp.float32))
        lax.fori_loop(0, TOT - NBUF + 1, body, init) if False else None
        T1 = TOT - NBUF + 1
        carry = lax.fori_loop(0, T1, body, init)
        for cp, pr in wcopies():
            cp.start(priority=pr)
        carry = lax.fori_loop(T1, TOT, body, carry)

        pltpu.make_async_copy(wg_v, wg_v, sw.at[3]).wait()
        gg = jnp.dot(xb, wg_v[...], preferred_element_type=jnp.float32)
        pltpu.make_async_copy(wu_v, wu_v, sw.at[4]).wait()
        uu = jnp.dot(xb, wu_v[...], preferred_element_type=jnp.float32)
        hh = (gg * jax.nn.sigmoid(gg) * uu).astype(jnp.bfloat16)
        pltpu.make_async_copy(wdT_v, wdT_v, sw.at[5]).wait()
        y = lax.dot_general(hh, wdT_v[...], (((1,), (1,)), ((), ())), preferred_element_type=jnp.float32)
        r = jnp.sum(xn.astype(jnp.float32) * wr_v[...].astype(jnp.float32), axis=-1, keepdims=True)
        res = x + xn.astype(jnp.float32) + y[0:1] * jax.nn.sigmoid(r)
        oc = jnp.broadcast_to(o_s[0:1, :], (8, HQ * DH)).astype(jnp.bfloat16)
        pltpu.make_async_copy(woT_v, woT_v, sw.at[6]).wait()
        a = lax.dot_general(oc, woT_v[...], (((1,), (1,)), ((), ())), preferred_element_type=jnp.float32)
        o_ref[...] = (res + a[0:1]).astype(o_ref.dtype)

    @jax.jit
    def fn(A_x, A_k_cache, A_v_cache, A_wq, A_wo, B_x, B_w_r, B_w_gate, B_w_up, B_w_down):
        hbm = pl.BlockSpec(memory_space=pltpu.HBM)
        out = pl.pallas_call(
            kernel,
            in_specs=[hbm] * 9,
            out_specs=pl.BlockSpec(memory_space=pltpu.VMEM),
            out_shape=jax.ShapeDtypeStruct((1, D), jnp.bfloat16),
            scratch_shapes=[
                pltpu.VMEM((1, D), jnp.bfloat16),
                pltpu.VMEM((1, D), jnp.bfloat16),
                pltpu.VMEM((D, HQ * DH), jnp.bfloat16),
                pltpu.VMEM((D, HQ * DH), jnp.bfloat16),
                pltpu.VMEM((D, F), jnp.bfloat16),
                pltpu.VMEM((D, F), jnp.bfloat16),
                pltpu.VMEM((D, F), jnp.bfloat16),
                pltpu.VMEM((NBUF, BS, DH), jnp.bfloat16),
                pltpu.VMEM((NBUF, BS, DH), jnp.bfloat16),
                pltpu.VMEM((HKV, 8, DH), jnp.bfloat16),
                pltpu.VMEM((8, HQ * DH), jnp.float32),
                pltpu.SemaphoreType.DMA((NBUF,)),
                pltpu.SemaphoreType.DMA((NBUF,)),
                pltpu.SemaphoreType.DMA((7,)),
            ],
            compiler_params=pltpu.CompilerParams(vmem_limit_bytes=100 * 1024 * 1024),
        )(A_x.reshape(1, D), A_k_cache, A_v_cache, A_wq, A_wo.T, B_w_r.reshape(1, D), B_w_gate, B_w_up, B_w_down.T)
        return out.reshape(1, 1, D)

    return fn


pallas_parallel_sum__gqa_block_cached__moe_arch_mod__decode_kernel = _make()
```

```python
import jax
import jax.numpy as jnp
from jax import lax
import jax.experimental.pallas as pl
import jax.experimental.pallas.tpu as pltpu

D = 448
HQ = 16
HKV = 8
DH = 256
SK = 65536
F = 1792
NT = (((1,), (1,)), ((), ()))


def _make(CH=64, BS=2048, NBUF=4, d=14, do_compute=True, W0=2, PER=2, scopes=False, issue_after=False):
    G = BS // CH
    NC = SK // BS
    TOT = HKV * NC
    NB = D // 16
    W1 = W0 + NB // PER
    IFF = W1 + NBUF
    FC = 256
    NF = F // FC
    L = NBUF - 1
    QI = (L - 1) * G // HKV
    assert QI * HKV == (L - 1) * G

    def kernel(x_hbm, k_hbm, v_hbm, wq_hbm, woT_hbm, wr_hbm, wg_hbm, wu_hbm, wdT_hbm, o_ref,
               x_v, wr_v, wq_v, woT_v, wg_v, wu_v, wdT_v, kb, vb, q_s, xb_s, res_s, sk, sv, sw):
        def pair(g, j, slot, c):
            c2 = (c + d) % G
            pltpu.make_async_copy(k_hbm.at[0, g, pl.ds(j * BS + c * CH, CH), :],
                                  kb.at[slot, pl.ds(c * CH, CH), :], sk.at[slot]).start(priority=0)
            pltpu.make_async_copy(v_hbm.at[0, g, pl.ds(j * BS + c2 * CH, CH), :],
                                  vb.at[slot, pl.ds(c2 * CH, CH), :], sv.at[slot]).start(priority=1)

        def start(i, slot):
            g = i // NC
            j = i % NC
            for c in range(G):
                pair(g, j, slot, c)

        def wait_all(buf, sem):
            pltpu.make_async_copy(buf, buf, sem).wait()

        def band(r):
            rs = pl.ds(r, 16)
            pltpu.make_async_copy(wg_hbm.at[rs, :], wg_v.at[rs, :], sw.at[3]).start(priority=0)
            pltpu.make_async_copy(wu_hbm.at[rs, :], wu_v.at[rs, :], sw.at[4]).start(priority=1)
            for p in range(4):
                sl = (rs, pl.ds(p * 1024, 1024))
                pltpu.make_async_copy(woT_hbm.at[sl], woT_v.at[sl], sw.at[6]).start(priority=p % 2)
            for p in range(2):
                sl = (rs, pl.ds(p * 896, 896))
                pltpu.make_async_copy(wdT_hbm.at[sl], wdT_v.at[sl], sw.at[5]).start(priority=p)

        pltpu.make_async_copy(x_hbm, x_v, sw.at[0]).start(priority=0)
        pltpu.make_async_copy(wr_hbm, wr_v, sw.at[1]).start(priority=1)

        @pl.loop(0, NB)
        def _(b):
            rs = pl.ds(pl.multiple_of(b * 16, 16), 16)
            for p in range(4):
                sl = (rs, pl.ds(p * 1024, 1024))
                pltpu.make_async_copy(wq_hbm.at[sl], wq_v.at[sl], sw.at[2]).start(priority=p % 2)

        wait_all(x_v, sw.at[0])
        x = x_v[...].astype(jnp.float32)
        mu = jnp.mean(x, axis=-1, keepdims=True)
        xc = x - mu
        var = jnp.mean(xc * xc, axis=-1, keepdims=True)
        xn = (xc / jnp.sqrt(var + 1e-5)).astype(jnp.bfloat16)
        xb_s[...] = jnp.broadcast_to(xn, (8, D))
        res_s[...] = jnp.broadcast_to(x + xn.astype(jnp.float32), (8, D))
        wait_all(wr_v, sw.at[1])
        r = jnp.sum(xn.astype(jnp.float32) * wr_v[...].astype(jnp.float32).reshape(1, D), axis=-1, keepdims=True)
        sr = jax.nn.sigmoid(r)

        @pl.loop(0, G // 4)
        def _(n):
            for t in range(4):
                pair(0, 0, 0, n * 4 + t)

        wait_all(wq_v, sw.at[2])

        @pl.loop(0, HKV)
        def _(h):
            for t in range(QI):
                n = G + h * QI + t
                pair(0, n // G, n // G, n % G)
            q = jnp.dot(xb_s[...], wq_v[:, pl.ds(pl.multiple_of(h * 512, 512), 512)],
                        preferred_element_type=jnp.float32)
            q = q.astype(jnp.bfloat16).astype(jnp.float32) * (DH ** -0.5)
            row = lax.broadcasted_iota(jnp.int32, (8, DH), 0)
            q_s[h] = jnp.where(row == 0, q[:, :DH], q[:, DH:]).astype(jnp.bfloat16)

        def body(i, carry):
            m_prev, l_prev, acc = carry
            slot = i % NBUF
            g = i // NC
            j = i % NC
            wait_all(kb.at[slot], sk.at[slot])
            wait_all(vb.at[slot], sv.at[slot])

            @pl.when(i + L < TOT)
            def _():
                start(i + L, (i + L) % NBUF)

            @pl.when(jnp.logical_and(i >= W0, i < W1))
            def _():
                for b in range(PER):
                    band(pl.multiple_of(((i - W0) * PER + b) * 16, 16))

            @pl.when(i == IFF - 1)
            def _():
                wait_all(wg_v, sw.at[3])
                wait_all(wu_v, sw.at[4])
                wait_all(wdT_v, sw.at[5])
                wait_all(woT_v, sw.at[6])

            @pl.when(jnp.logical_and(i >= IFF, i < IFF + NF))
            def _():
                cs = pl.ds(pl.multiple_of((i - IFF) * FC, FC), FC)
                gg = jnp.dot(xb_s[...], wg_v[:, cs], preferred_element_type=jnp.float32)
                uu = jnp.dot(xb_s[...], wu_v[:, cs], preferred_element_type=jnp.float32)
                hh = (gg * jax.nn.sigmoid(gg) * uu).astype(jnp.bfloat16)
                res_s[...] += sr * lax.dot_general(hh, wdT_v[:, cs], NT, preferred_element_type=jnp.float32)

            if not do_compute:
                return carry
            first = j == 0
            m_prev = jnp.where(first, -jnp.inf, m_prev)
            l_prev = jnp.where(first, 0.0, l_prev)
            acc = jnp.where(first, 0.0, acc)
            s = lax.dot_general(q_s[g], kb[slot], NT, preferred_element_type=jnp.float32)
            m_new = jnp.maximum(m_prev, jnp.max(s, axis=-1, keepdims=True))
            alpha = jnp.exp(m_prev - m_new)
            p = jnp.exp(s - m_new)
            l_new = alpha * l_prev + jnp.sum(p, axis=-1, keepdims=True)
            acc = alpha * acc + jnp.dot(p.astype(jnp.bfloat16), vb[slot], preferred_element_type=jnp.float32)

            @pl.when(j == NC - 1)
            def _():
                o = acc / l_new
                oc = jnp.concatenate([o[0:1], o[1:2]], axis=-1).astype(jnp.bfloat16)
                oc = jnp.broadcast_to(oc, (8, 512))
                w = woT_v[:, pl.ds(pl.multiple_of(g * 512, 512), 512)]
                res_s[...] += lax.dot_general(oc, w, NT, preferred_element_type=jnp.float32)
            return m_new, l_new, acc

        init = (jnp.zeros((8, 1), jnp.float32), jnp.zeros((8, 1), jnp.float32), jnp.zeros((8, DH), jnp.float32))
        lax.fori_loop(0, TOT, body, init)
        o_ref[...] = res_s[0:1, :].astype(o_ref.dtype)

    @jax.jit
    def fn(A_x, A_k_cache, A_v_cache, A_wq, A_wo, B_x, B_w_r, B_w_gate, B_w_up, B_w_down):
        hbm = pl.BlockSpec(memory_space=pltpu.HBM)
        out = pl.pallas_call(
            kernel,
            in_specs=[hbm] * 9,
            out_specs=pl.BlockSpec(memory_space=pltpu.VMEM),
            out_shape=jax.ShapeDtypeStruct((1, D), jnp.bfloat16),
            scratch_shapes=[
                pltpu.VMEM((1, D), jnp.bfloat16),
                pltpu.VMEM((D,), jnp.bfloat16),
                pltpu.VMEM((D, HQ * DH), jnp.bfloat16),
                pltpu.VMEM((D, HQ * DH), jnp.bfloat16),
                pltpu.VMEM((D, F), jnp.bfloat16),
                pltpu.VMEM((D, F), jnp.bfloat16),
                pltpu.VMEM((D, F), jnp.bfloat16),
                pltpu.VMEM((NBUF, BS, DH), jnp.bfloat16),
                pltpu.VMEM((NBUF, BS, DH), jnp.bfloat16),
                pltpu.VMEM((HKV, 8, DH), jnp.bfloat16),
                pltpu.VMEM((8, D), jnp.bfloat16),
                pltpu.VMEM((8, D), jnp.float32),
                pltpu.SemaphoreType.DMA((NBUF,)),
                pltpu.SemaphoreType.DMA((NBUF,)),
                pltpu.SemaphoreType.DMA((7,)),
            ],
            compiler_params=pltpu.CompilerParams(vmem_limit_bytes=100 * 1024 * 1024),
        )(A_x.reshape(1, D), A_k_cache, A_v_cache, A_wq, A_wo.T, B_w_r, B_w_gate, B_w_up, B_w_down.T)
        return out.reshape(1, 1, D)

    return fn


pallas_parallel_sum__gqa_block_cached__moe_arch_mod__decode_kernel = _make()
```

```python
import jax
import jax.numpy as jnp
from jax import lax
import jax.experimental.pallas as pl
import jax.experimental.pallas.tpu as pltpu

D, HQ, HKV, DH, F = 448, 16, 8, 256, 1792
NT = (((1,), (1,)), ((), ()))
F32, BF16 = jnp.float32, jnp.bfloat16


def _make(SK=65536, CH=64, BS=1024, NBUF=6, ROT=14, W0=2, PER=1):
    G = BS // CH
    NC = SK // BS
    TOT = HKV * NC
    L = NBUF - 1
    NB = D // 16
    W1 = W0 + NB // PER
    IFF = W1 + NBUF
    FC = 256
    NF = F // FC
    QI = (L - 1) * G // HKV
    assert QI * HKV == (L - 1) * G and NB % PER == 0 and G % 4 == 0
    assert IFF <= NC and IFF + NF <= TOT

    def kernel(x_hbm, k_hbm, v_hbm, wq_hbm, woT_hbm, wr_hbm, wg_hbm, wu_hbm, wdT_hbm, o_ref,
               x_v, wr_v, wq_v, woT_v, wg_v, wu_v, wdT_v, kb, vb, q_s, xb_s, res_s, sk, sv, sw):
        def copy(src, dst, sl, sem, prio):
            pltpu.make_async_copy(src.at[sl], dst.at[sl], sem).start(priority=prio)

        def pair(g, j, slot, c):
            for src, dst, sem, cc, prio in ((k_hbm, kb, sk, c, 0), (v_hbm, vb, sv, (c + ROT) % G, 1)):
                pltpu.make_async_copy(src.at[0, g, pl.ds(j * BS + cc * CH, CH), :],
                                      dst.at[slot, pl.ds(cc * CH, CH), :],
                                      sem.at[slot]).start(priority=prio)

        def wait_all(buf, sem):
            pltpu.make_async_copy(buf, buf, sem).wait()

        def rows(b):
            return pl.ds(pl.multiple_of(b * 16, 16), 16)

        pltpu.make_async_copy(x_hbm, x_v, sw.at[0]).start(priority=0)
        pltpu.make_async_copy(wr_hbm, wr_v, sw.at[1]).start(priority=1)

        @pl.loop(0, NB)
        def _(b):
            for p in range(4):
                copy(wq_hbm, wq_v, (rows(b), pl.ds(p * 1024, 1024)), sw.at[2], p % 2)

        wait_all(x_v, sw.at[0])
        x = x_v[...].astype(F32)
        xc = x - jnp.mean(x, axis=-1, keepdims=True)
        var = jnp.mean(xc * xc, axis=-1, keepdims=True)
        xn = (xc / jnp.sqrt(var + 1e-5)).astype(BF16)
        xb_s[...] = jnp.broadcast_to(xn, (8, D))
        res_s[...] = jnp.broadcast_to(x + xn.astype(F32), (8, D))
        wait_all(wr_v, sw.at[1])
        r = jnp.sum(xn.astype(F32) * wr_v[...].astype(F32).reshape(1, D), axis=-1, keepdims=True)
        gate = jax.nn.sigmoid(r)

        @pl.loop(0, G // 4)
        def _(n):
            for t in range(4):
                pair(0, 0, 0, n * 4 + t)

        wait_all(wq_v, sw.at[2])

        @pl.loop(0, HKV)
        def _(h):
            for t in range(QI):
                n = G + h * QI + t
                pair(0, n // G, n // G, n % G)
            q = jnp.dot(xb_s[...], wq_v[:, pl.ds(pl.multiple_of(h * 512, 512), 512)],
                        preferred_element_type=F32)
            q = q.astype(BF16).astype(F32) * (DH ** -0.5)
            row = lax.broadcasted_iota(jnp.int32, (8, DH), 0)
            q_s[h] = jnp.where(row == 0, q[:, :DH], q[:, DH:]).astype(BF16)

        def body(i, carry):
            m_prev, l_prev, acc = carry
            slot = i % NBUF
            g = i // NC
            j = i % NC
            wait_all(kb.at[slot], sk.at[slot])
            wait_all(vb.at[slot], sv.at[slot])

            @pl.when(i + L < TOT)
            def _():
                n = i + L
                for c in range(G):
                    pair(n // NC, n % NC, n % NBUF, c)

            @pl.when(jnp.logical_and(i >= W0, i < W1))
            def _():
                for b in range(PER):
                    rs = rows((i - W0) * PER + b)
                    copy(wg_hbm, wg_v, (rs, slice(None)), sw.at[3], 0)
                    copy(wu_hbm, wu_v, (rs, slice(None)), sw.at[4], 1)
                    for p in range(4):
                        copy(woT_hbm, woT_v, (rs, pl.ds(p * 1024, 1024)), sw.at[6], p % 2)
                    for p in range(2):
                        copy(wdT_hbm, wdT_v, (rs, pl.ds(p * 896, 896)), sw.at[5], p)

            @pl.when(i == IFF - 1)
            def _():
                wait_all(wg_v, sw.at[3])
                wait_all(wu_v, sw.at[4])
                wait_all(wdT_v, sw.at[5])
                wait_all(woT_v, sw.at[6])

            @pl.when(jnp.logical_and(i >= IFF, i < IFF + NF))
            def _():
                cs = pl.ds(pl.multiple_of((i - IFF) * FC, FC), FC)
                gg = jnp.dot(xb_s[...], wg_v[:, cs], preferred_element_type=F32)
                uu = jnp.dot(xb_s[...], wu_v[:, cs], preferred_element_type=F32)
                hh = (gg * jax.nn.sigmoid(gg) * uu).astype(BF16)
                res_s[...] += gate * lax.dot_general(hh, wdT_v[:, cs], NT, preferred_element_type=F32)

            first = j == 0
            m_prev = jnp.where(first, -jnp.inf, m_prev)
            l_prev = jnp.where(first, 0.0, l_prev)
            acc = jnp.where(first, 0.0, acc)
            s = lax.dot_general(q_s[g], kb[slot], NT, preferred_element_type=F32)
            m_new = jnp.maximum(m_prev, jnp.max(s, axis=-1, keepdims=True))
            alpha = jnp.exp(m_prev - m_new)
            p = jnp.exp(s - m_new)
            l_new = alpha * l_prev + jnp.sum(p, axis=-1, keepdims=True)
            acc = alpha * acc + jnp.dot(p.astype(BF16), vb[slot], preferred_element_type=F32)

            @pl.when(j == NC - 1)
            def _():
                o = acc / l_new
                oc = jnp.concatenate([o[0:1], o[1:2]], axis=-1).astype(BF16)
                w = woT_v[:, pl.ds(pl.multiple_of(g * 512, 512), 512)]
                res_s[...] += lax.dot_general(jnp.broadcast_to(oc, (8, 512)), w, NT,
                                              preferred_element_type=F32)

            return m_new, l_new, acc

        init = (jnp.zeros((8, 1), F32), jnp.zeros((8, 1), F32), jnp.zeros((8, DH), F32))
        lax.fori_loop(0, TOT, body, init)
        o_ref[...] = res_s[0:1, :].astype(o_ref.dtype)

    @jax.jit
    def fn(A_x, A_k_cache, A_v_cache, A_wq, A_wo, B_x, B_w_r, B_w_gate, B_w_up, B_w_down):
        del B_x
        out = pl.pallas_call(
            kernel,
            in_specs=[pl.BlockSpec(memory_space=pltpu.HBM)] * 9,
            out_specs=pl.BlockSpec(memory_space=pltpu.VMEM),
            out_shape=jax.ShapeDtypeStruct((1, D), BF16),
            scratch_shapes=[
                pltpu.VMEM((1, D), BF16), pltpu.VMEM((D,), BF16),
                pltpu.VMEM((D, HQ * DH), BF16), pltpu.VMEM((D, HQ * DH), BF16),
                pltpu.VMEM((D, F), BF16), pltpu.VMEM((D, F), BF16), pltpu.VMEM((D, F), BF16),
                pltpu.VMEM((NBUF, BS, DH), BF16), pltpu.VMEM((NBUF, BS, DH), BF16),
                pltpu.VMEM((HKV, 8, DH), BF16), pltpu.VMEM((8, D), BF16), pltpu.VMEM((8, D), F32),
                pltpu.SemaphoreType.DMA((NBUF,)), pltpu.SemaphoreType.DMA((NBUF,)),
                pltpu.SemaphoreType.DMA((7,)),
            ],
            compiler_params=pltpu.CompilerParams(vmem_limit_bytes=64 * 1024 * 1024),
        )(A_x.reshape(1, D), A_k_cache, A_v_cache, A_wq, A_wo.T, B_w_r, B_w_gate, B_w_up, B_w_down.T)
        return out.reshape(1, 1, D)

    return fn


pallas_parallel_sum__gqa_block_cached__moe_arch_mod__decode_kernel = _make()
```
